```python
import jax
import jax.numpy as jnp

def _softmax(x, axis=-1):
    return jax.nn.softmax(x, axis=axis)
def _gelu(x):
    return jax.nn.gelu(x, approximate=True)
def _silu(x):
    return jax.nn.silu(x)
def _sigmoid(x):
    return jax.nn.sigmoid(x)
def _layernorm(x, axis=-1, eps=1e-5):
    m = jnp.mean(x, axis=axis, keepdims=True)
    v = jnp.var(x, axis=axis, keepdims=True)
    return (x - m) / jnp.sqrt(v + eps)
def _scatter_add(tgt, idx, src, axis=0):
    return tgt.at[idx].add(src)
def _segment_sum(src, seg, n):
    return jax.ops.segment_sum(src, seg, n)
class _Rng:
    def __init__(self, key):
        self._k = key
    def _next(self):
        self._k, sub = jax.random.split(self._k)
        return sub
    def normal(self, shape):
        return jax.random.normal(self._next(), shape, dtype=jnp.bfloat16)
    def randint(self, lo, hi, shape):
        return jax.random.randint(self._next(), shape, lo, hi, dtype=jnp.int32)
    def uniform(self, shape, lo=0.0, hi=1.0):
        return jax.random.uniform(self._next(), shape, jnp.bfloat16, lo, hi)
    def permutation(self, n):
        return jax.random.permutation(self._next(), n)


kernel_name = 'standalone__standard_2d_1d_3d_conv__vision'

def setup_inputs():
    _rng = _Rng(jax.random.key(int.from_bytes(__import__("os").urandom(4), "little")))
    _w = (lambda a: (lambda t: t.astype(jnp.bfloat16) if jnp.issubdtype(t.dtype, jnp.floating) else t)(jnp.asarray(a)))
    H = W = 384
    C = 384
    K = 1
    return {
        "x": _w((lambda *s: _rng.normal(s) * 0.05)(1, H, W, C)),
        "w": _w((lambda *s: _rng.normal(s) * 0.05)(K, K, C, C)),
        "b": _w((lambda *s: _rng.normal(s) * 0.05)(C)),
    }

def reference(x, w, b):
    B, H, W, Cin = x.shape
    K = w.shape[0]
    pl = (K - 1) // 2
    pr = K // 2
    xp = jnp.pad(x, ((0, 0), (pl, pr), (pl, pr), (0, 0)))
    out = sum(
        jnp.einsum('bhwc,cd->bhwd', xp[:, i:i+H, j:j+W, :], w[i, j])
        for i in range(K) for j in range(K)
    )
    return out + b[None, None, None, :]
```

```python
import jax
import jax.numpy as jnp
import jax.experimental.pallas as pl
import jax.experimental.pallas.tpu as pltpu

T = 6
RR = 32
WR = 48
Q = 192
PRE = 31
KA = 11
EXTRA = 1
LA = 1
W0 = 64
KB = 7


@jax.jit
def pallas_standalone__standard_2d_1d_3d_conv__vision_kernel(
    x: jax.Array,
    w: jax.Array,
    b: jax.Array,
):
    B, H, W, Cin = x.shape
    assert w.shape[0] == 1 and w.shape[1] == 1
    Cout = w.shape[-1]
    assert Cin == Cout
    M = B * H * W
    S = M // T
    ha = T // 2
    nround, nwin, nchunk = S // RR, S // WR, S // Q
    rpc, wpc = Q // RR, Q // WR
    assert M % T == 0 and S % Q == 0 and Q % RR == 0 and Q % WR == 0
    assert (nround - PRE) % KA == 0 and KA >= rpc
    nA = (nround - PRE) // KA
    nB0 = nA + EXTRA
    wend = W0 + KB * (nchunk - nB0)
    assert wend <= nwin and W0 <= nB0 * wpc and nB0 <= nchunk - LA
    assert all(W0 + KB * (i + 1 - nB0) <= wpc * (i + 1) for i in range(nB0, nchunk))

    def kernel_function(x_hbm, w_ref, b_ref, o_hbm, buf, rsem, wsem):
        def start_rounds(lo, n):
            def body(t, c):
                j = lo + t
                rows = pl.ds(pl.multiple_of(j * RR, RR), RR)
                for g in range(2):
                    idx = (pl.ds(g * ha, ha), rows, slice(None))
                    pltpu.make_async_copy(
                        x_hbm.at[idx], buf.at[idx], rsem.at[j // rpc]
                    ).start(priority=g)
                return c
            jax.lax.fori_loop(0, n, body, 0)

        def chunk_idx(i):
            return (slice(None), pl.ds(pl.multiple_of(i * Q, Q), Q), slice(None))

        def wait_chunk(i):
            v = buf.at[chunk_idx(i)]
            pltpu.make_async_copy(v, v, rsem.at[i]).wait()

        def start_wins(lo, n):
            def body(t, c):
                rows = pl.ds(pl.multiple_of((lo + t) * WR, WR), WR)
                idx = (slice(None), rows, slice(None))
                pltpu.make_async_copy(buf.at[idx], o_hbm.at[idx], wsem.at[0]).start()
                return c
            jax.lax.fori_loop(0, n, body, 0)

        def comp(i):
            idx = chunk_idx(i)
            xv = buf[idx].reshape(T * Q, Cin)
            acc = jnp.dot(xv, w_ref[...], preferred_element_type=jnp.float32)
            y = (acc + b_ref[...].astype(jnp.float32)).astype(buf.dtype)
            buf[idx] = y.reshape(T, Q, Cout)

        def loop_read(i, c):
            start_rounds(PRE + i * KA, KA)
            wait_chunk(i)
            comp(i)
            return c

        def loop_extra(i, c):
            wait_chunk(i)
            comp(i)
            return c

        def loop_wait(i, c):
            wait_chunk(i)
            return c

        def loop_write(i, c):
            comp(i)
            start_wins(W0 + (i - nB0) * KB, KB)
            return c

        start_rounds(0, PRE)
        jax.lax.fori_loop(0, nA, loop_read, 0)
        jax.lax.fori_loop(nA, nB0, loop_extra, 0)
        jax.lax.fori_loop(nB0, nchunk - LA, loop_wait, 0)
        start_wins(0, W0)
        jax.lax.fori_loop(nchunk - LA, nchunk, loop_wait, 0)
        jax.lax.fori_loop(nB0, nchunk, loop_write, 0)
        start_wins(wend, nwin - wend)
        pltpu.make_async_copy(buf, o_hbm, wsem.at[0]).wait()

    out = pl.pallas_call(
        kernel_function,
        in_specs=[
            pl.BlockSpec(memory_space=pl.ANY),
            pl.BlockSpec(memory_space=pltpu.VMEM),
            pl.BlockSpec(memory_space=pltpu.VMEM),
        ],
        out_specs=pl.BlockSpec(memory_space=pl.ANY),
        out_shape=jax.ShapeDtypeStruct((T, S, Cout), x.dtype),
        scratch_shapes=[
            pltpu.VMEM((T, S, Cin), x.dtype),
            pltpu.SemaphoreType.DMA((nchunk,)),
            pltpu.SemaphoreType.DMA((1,)),
        ],
        compiler_params=pltpu.CompilerParams(
            vmem_limit_bytes=125 * 1024 * 1024,
            disable_bounds_checks=True,
        ),
    )(x.reshape(T, S, Cin), w.reshape(Cin, Cout), b.reshape(1, Cout))
    return out.reshape(B, H, W, Cout)
```

```python
import jax
import jax.numpy as jnp
import jax.experimental.pallas as pl
import jax.experimental.pallas.tpu as pltpu

TR = 8
RR = 24
QR = 144
TW = 6
WR = 48
QW = 192
SKIP = 8
W0 = 64
KB = 6
WSPLIT = 4


@jax.jit
def pallas_standalone__standard_2d_1d_3d_conv__vision_kernel(
    x: jax.Array,
    w: jax.Array,
    b: jax.Array,
):
    B, H, W, Cin = x.shape
    Cout = w.shape[-1]
    assert w.shape[:2] == (1, 1) and Cin == Cout
    M = B * H * W
    SR, SW = M // (2 * TR), M // (2 * TW)
    assert M % (2 * TR) == 0 and SR % QR == 0 and QR % RR == 0
    assert M % (2 * TW) == 0 and SW % QW == 0 and QW % WR == 0
    ha = TR // 2
    ncr = SR // QR
    ncw = SW // QW
    nwh = SW // WR
    nchunk = 2 * ncr
    pre = ncr // SKIP
    assert ncr % SKIP == 0 and pre >= 1
    wend = W0 + KB * ncw
    assert W0 <= nwh and wend <= 2 * nwh
    assert all(W0 + KB * n <= nwh + (QW // WR) * n for n in range(1, ncw + 1))
    wrows = Cin // WSPLIT

    def kernel_function(x_hbm, w_hbm, b_hbm, o_hbm,
                        buf, w_ref, b_ref, bf_ref, rsem, wsem, psem):
        bufw = buf.reshape(2 * TW, SW, Cout)

        def split(c, n):
            h = (c >= n).astype(jnp.int32)
            return h, c - h * n

        def start_chunk(c):
            h, cc = split(c, ncr)
            for t in range(QR // RR):
                rows = pl.ds(pl.multiple_of(cc * QR + t * RR, RR), RR)
                for g in range(2):
                    idx = (pl.ds(h * TR + g * ha, ha), rows, slice(None))
                    pltpu.make_async_copy(
                        x_hbm.at[idx], buf.at[idx], rsem.at[c]
                    ).start(priority=g)

        def wait_chunk(c):
            h, cc = split(c, ncr)
            v = buf.at[pl.ds(h * TR, TR), pl.ds(pl.multiple_of(cc * QR, QR), QR), :]
            pltpu.make_async_copy(v, v, rsem.at[c]).wait()

        def start_write(k):
            h, kk = split(k, nwh)
            idx = (pl.ds(h * TW, TW), pl.ds(pl.multiple_of(kk * WR, WR), WR), slice(None))
            pltpu.make_async_copy(bufw.at[idx], o_hbm.at[idx], wsem.at[0]).start()

        def matmul_in_place(ref, idx):
            xv = ref[idx]
            acc = jnp.dot(xv.reshape(-1, Cin), w_ref[...],
                          preferred_element_type=jnp.float32)
            ref[idx] = (acc + bf_ref[...]).astype(ref.dtype).reshape(xv.shape)

        def loop(lo, hi, fn):
            def body(i, c):
                fn(i)
                return c
            jax.lax.fori_loop(lo, hi, body, 0)

        w_copies = [
            pltpu.make_async_copy(w_hbm.at[pl.ds(k * wrows, wrows)],
                                  w_ref.at[pl.ds(k * wrows, wrows)], psem.at[0])
            for k in range(WSPLIT)
        ]
        b_copy = pltpu.make_async_copy(b_hbm, b_ref, psem.at[1])
        for k, cp in enumerate(w_copies):
            cp.start(priority=k % 2)
        b_copy.start()
        loop(0, pre, start_chunk)
        b_copy.wait()
        bf_ref[...] = b_ref[...].astype(jnp.float32).reshape(1, Cout)
        for cp in w_copies:
            cp.wait()

        def step_a(i, nxt):
            wait_chunk(i)
            start_chunk(nxt)
            two = jax.lax.rem(i, SKIP) != SKIP - 1

            @pl.when(two)
            def _():
                start_chunk(nxt + 1)

            matmul_in_place(
                buf, (pl.ds(0, TR), pl.ds(pl.multiple_of(i * QR, QR), QR), slice(None)))
            return nxt + 1 + two.astype(jnp.int32)

        jax.lax.fori_loop(0, ncr, step_a, jnp.int32(pre))

        loop(ncr, nchunk - 1, wait_chunk)
        loop(0, W0, start_write)
        wait_chunk(jnp.int32(nchunk - 1))

        def step_b(i):
            matmul_in_place(
                bufw, (pl.ds(TW, TW), pl.ds(pl.multiple_of(i * QW, QW), QW), slice(None)))
            for t in range(KB):
                start_write(W0 + i * KB + t)

        loop(0, ncw, step_b)
        loop(wend, 2 * nwh, start_write)
        pltpu.make_async_copy(bufw, o_hbm, wsem.at[0]).wait()

    out = pl.pallas_call(
        kernel_function,
        in_specs=[pl.BlockSpec(memory_space=pl.ANY)] * 3,
        out_specs=pl.BlockSpec(memory_space=pl.ANY),
        out_shape=jax.ShapeDtypeStruct((2 * TW, SW, Cout), x.dtype),
        scratch_shapes=[
            pltpu.VMEM((2 * TR, SR, Cin), x.dtype),
            pltpu.VMEM((Cin, Cout), w.dtype),
            pltpu.VMEM(b.shape, b.dtype),
            pltpu.VMEM((1, Cout), jnp.float32),
            pltpu.SemaphoreType.DMA((nchunk,)),
            pltpu.SemaphoreType.DMA((1,)),
            pltpu.SemaphoreType.DMA((2,)),
        ],
        compiler_params=pltpu.CompilerParams(
            vmem_limit_bytes=125 * 1024 * 1024,
            disable_bounds_checks=True,
            disable_semaphore_checks=True,
        ),
    )(x.reshape(2 * TR, SR, Cin), w.reshape(Cin, Cout), b)
    return out.reshape(B, H, W, Cout)
```

```python
import jax
import jax.numpy as jnp
import jax.experimental.pallas as pl
import jax.experimental.pallas.tpu as pltpu

T = 6
RR = 16
WR = 48
Q = 192
PRE = 3
LR = 6
W0 = 64
KB = 6
WSPLIT = 4


@jax.jit
def pallas_standalone__standard_2d_1d_3d_conv__vision_kernel(
    x: jax.Array,
    w: jax.Array,
    b: jax.Array,
):
    B, H, W, Cin = x.shape
    Cout = w.shape[-1]
    assert w.shape[:2] == (1, 1) and Cin == Cout
    M = B * H * W
    S = M // (2 * T)
    assert M % (2 * T) == 0 and S % Q == 0 and Q % RR == 0 and Q % WR == 0
    nc = S // Q
    nwh = S // WR
    rpc, wpc = Q // RR, Q // WR
    n_a = nc - 2
    n_b = 2 * nc - n_a
    wend = W0 + KB * n_b
    assert 0 < LR < rpc and 2 <= PRE <= nc - 1
    assert W0 <= n_a * wpc and wend <= 2 * nwh
    assert all(W0 + KB * n <= (n_a + n) * wpc for n in range(1, n_b + 1))
    wrows = Cin // WSPLIT
    last = (nc - 1) * Q
    tail = S - LR * RR

    def kernel_function(x_hbm, w_hbm, b_hbm, o_hbm,
                        buf, w_ref, b_ref, bf_ref, rsem, hsem, lsem, wsem, psem):
        def split(c, n):
            h = (c >= n).astype(jnp.int32)
            return h, c - h * n

        def start_round(row, sems):
            for h in range(2):
                idx = (pl.ds(h * T, T), pl.ds(row, RR), slice(None))
                pltpu.make_async_copy(
                    x_hbm.at[idx], buf.at[idx], sems[h]).start(priority=h)

        def start_chunk(c):
            for t in range(rpc):
                start_round(pl.multiple_of(c * Q + t * RR, RR),
                            (rsem.at[c], hsem.at[0]))

        def start_last_chunk():
            for row in range(last, S, RR):
                sem = lsem.at[0 if row < tail else 1]
                start_round(row, (sem, sem))

        def wait_rows(streams, rows, sem):
            v = buf.at[streams, rows, :]
            pltpu.make_async_copy(v, v, sem).wait()

        def start_write(k):
            h, kk = split(k, nwh)
            idx = (pl.ds(h * T, T), pl.ds(pl.multiple_of(kk * WR, WR), WR), slice(None))
            pltpu.make_async_copy(buf.at[idx], o_hbm.at[idx], wsem.at[0]).start()

        def matmul_in_place(h, c):
            idx = (pl.ds(h * T, T), pl.ds(pl.multiple_of(c * Q, Q), Q), slice(None))
            acc = jnp.dot(buf[idx].reshape(T * Q, Cin), w_ref[...],
                          preferred_element_type=jnp.float32)
            buf[idx] = (acc + bf_ref[...]).astype(buf.dtype).reshape(T, Q, Cout)

        def loop(lo, hi, fn):
            def body(i, c):
                fn(i)
                return c
            jax.lax.fori_loop(lo, hi, body, 0)

        half0, half1, both = pl.ds(0, T), pl.ds(T, T), pl.ds(0, 2 * T)

        w_copies = [
            pltpu.make_async_copy(w_hbm.at[pl.ds(k * wrows, wrows)],
                                  w_ref.at[pl.ds(k * wrows, wrows)], psem.at[0])
            for k in range(WSPLIT)
        ]
        b_copy = pltpu.make_async_copy(b_hbm, b_ref, psem.at[1])
        for k, cp in enumerate(w_copies):
            cp.start(priority=k % 2)
        b_copy.start()
        loop(0, PRE, start_chunk)
        b_copy.wait()
        bf_ref[...] = b_ref[...].astype(jnp.float32).reshape(1, Cout)
        for cp in w_copies:
            cp.wait()

        def step_a(i):
            @pl.when(i + PRE < nc - 1)
            def _():
                start_chunk(i + PRE)

            @pl.when(i + PRE == nc - 1)
            def _():
                start_last_chunk()

            wait_rows(half0, pl.ds(pl.multiple_of(i * Q, Q), Q), rsem.at[i])
            matmul_in_place(0, i)

        loop(0, n_a, step_a)

        wait_rows(half0, pl.ds(n_a * Q, Q), rsem.at[n_a])
        wait_rows(half1, pl.ds(0, last), hsem.at[0])
        wait_rows(both, pl.ds(last, tail - last), lsem.at[0])
        loop(0, W0, start_write)
        wait_rows(both, pl.ds(tail, S - tail), lsem.at[1])

        def step_b(i):
            matmul_in_place(*split(n_a + i, nc))
            for t in range(KB):
                start_write(W0 + i * KB + t)

        loop(0, n_b, step_b)
        loop(wend, 2 * nwh, start_write)
        pltpu.make_async_copy(buf, o_hbm, wsem.at[0]).wait()

    out = pl.pallas_call(
        kernel_function,
        in_specs=[pl.BlockSpec(memory_space=pl.ANY)] * 3,
        out_specs=pl.BlockSpec(memory_space=pl.ANY),
        out_shape=jax.ShapeDtypeStruct((2 * T, S, Cout), x.dtype),
        scratch_shapes=[
            pltpu.VMEM((2 * T, S, Cin), x.dtype),
            pltpu.VMEM((Cin, Cout), w.dtype),
            pltpu.VMEM(b.shape, b.dtype),
            pltpu.VMEM((1, Cout), jnp.float32),
            pltpu.SemaphoreType.DMA((nc - 1,)),
            pltpu.SemaphoreType.DMA((1,)),
            pltpu.SemaphoreType.DMA((2,)),
            pltpu.SemaphoreType.DMA((1,)),
            pltpu.SemaphoreType.DMA((2,)),
        ],
        compiler_params=pltpu.CompilerParams(
            vmem_limit_bytes=116 * 1024 * 1024,
            disable_bounds_checks=True,
            disable_semaphore_checks=True,
        ),
    )(x.reshape(2 * T, S, Cin), w.reshape(Cin, Cout), b)
    return out.reshape(B, H, W, Cout)
```

```python
import jax
import jax.numpy as jnp
import jax.experimental.pallas as pl
import jax.experimental.pallas.tpu as pltpu

T = 6
RR = 8
WR = 48
Q = 192
PRE = 2
LR = 12
W0 = 64
KB = 6
WSPLIT = 8


@jax.jit
def pallas_standalone__standard_2d_1d_3d_conv__vision_kernel(
    x: jax.Array,
    w: jax.Array,
    b: jax.Array,
):
    B, H, W, Cin = x.shape
    Cout = w.shape[-1]
    assert w.shape[:2] == (1, 1) and Cin == Cout
    M = B * H * W
    S = M // (2 * T)
    assert M % (2 * T) == 0 and S % Q == 0 and Q % RR == 0 and Q % WR == 0
    nc = S // Q
    nwh = S // WR
    rpc, wpc = Q // RR, Q // WR
    n_a = nc - 2
    n_b = 2 * nc - n_a
    wend = W0 + KB * n_b
    assert 0 < LR < rpc and 2 <= PRE <= nc - 1
    assert W0 <= n_a * wpc and wend <= 2 * nwh
    assert all(W0 + KB * n <= (n_a + n) * wpc for n in range(1, n_b + 1))
    wrows = Cin // WSPLIT
    last = (nc - 1) * Q
    tail = S - LR * RR

    def kernel_function(x_hbm, w_hbm, b_hbm, o_hbm,
                        buf, w_ref, b_ref, bf_ref, rsem, hsem, lsem, wsem, psem):
        def split(c, n):
            h = (c >= n).astype(jnp.int32)
            return h, c - h * n

        def start_round(row, sems):
            for h in range(2):
                idx = (pl.ds(h * T, T), pl.ds(row, RR), slice(None))
                pltpu.make_async_copy(
                    x_hbm.at[idx], buf.at[idx], sems[h]).start(priority=h)

        def start_chunk(c):
            for t in range(rpc):
                start_round(pl.multiple_of(c * Q + t * RR, RR),
                            (rsem.at[c], hsem.at[0]))

        def start_last_chunk():
            for row in range(last, S, RR):
                sem = lsem.at[0 if row < tail else 1]
                start_round(row, (sem, sem))

        def wait_rows(streams, rows, sem):
            v = buf.at[streams, rows, :]
            pltpu.make_async_copy(v, v, sem).wait()

        def start_write(k):
            h, kk = split(k, nwh)
            idx = (pl.ds(h * T, T), pl.ds(pl.multiple_of(kk * WR, WR), WR), slice(None))
            pltpu.make_async_copy(buf.at[idx], o_hbm.at[idx], wsem.at[0]).start()

        def matmul_in_place(h, c):
            idx = (pl.ds(h * T, T), pl.ds(pl.multiple_of(c * Q, Q), Q), slice(None))
            acc = jnp.dot(buf[idx].reshape(T * Q, Cin), w_ref[...],
                          preferred_element_type=jnp.float32)
            buf[idx] = (acc + bf_ref[...]).astype(buf.dtype).reshape(T, Q, Cout)

        def loop(lo, hi, fn):
            def body(i, c):
                fn(i)
                return c
            jax.lax.fori_loop(lo, hi, body, 0)

        half0, half1, both = pl.ds(0, T), pl.ds(T, T), pl.ds(0, 2 * T)

        w_copies = [
            pltpu.make_async_copy(w_hbm.at[pl.ds(k * wrows, wrows)],
                                  w_ref.at[pl.ds(k * wrows, wrows)], psem.at[0])
            for k in range(WSPLIT)
        ]
        b_copy = pltpu.make_async_copy(b_hbm, b_ref, psem.at[1])
        for k, cp in enumerate(w_copies):
            cp.start(priority=k % 2)
        b_copy.start()
        loop(0, PRE, start_chunk)
        b_copy.wait()
        bf_ref[...] = b_ref[...].astype(jnp.float32).reshape(1, Cout)
        for cp in w_copies:
            cp.wait()

        def step_a(i):
            @pl.when(i + PRE < nc - 1)
            def _():
                start_chunk(i + PRE)

            @pl.when(i + PRE == nc - 1)
            def _():
                start_last_chunk()

            wait_rows(half0, pl.ds(pl.multiple_of(i * Q, Q), Q), rsem.at[i])
            matmul_in_place(0, i)

        loop(0, n_a, step_a)

        wait_rows(half0, pl.ds(n_a * Q, Q), rsem.at[n_a])
        wait_rows(half1, pl.ds(0, last), hsem.at[0])
        wait_rows(both, pl.ds(last, tail - last), lsem.at[0])
        loop(0, W0, start_write)
        wait_rows(both, pl.ds(tail, S - tail), lsem.at[1])

        def step_b(i):
            matmul_in_place(*split(n_a + i, nc))
            for t in range(KB):
                start_write(W0 + i * KB + t)

        loop(0, n_b, step_b)
        loop(wend, 2 * nwh, start_write)
        pltpu.make_async_copy(buf, o_hbm, wsem.at[0]).wait()

    out = pl.pallas_call(
        kernel_function,
        in_specs=[pl.BlockSpec(memory_space=pl.ANY)] * 3,
        out_specs=pl.BlockSpec(memory_space=pl.ANY),
        out_shape=jax.ShapeDtypeStruct((2 * T, S, Cout), x.dtype),
        scratch_shapes=[
            pltpu.VMEM((2 * T, S, Cin), x.dtype),
            pltpu.VMEM((Cin, Cout), w.dtype),
            pltpu.VMEM(b.shape, b.dtype),
            pltpu.VMEM((1, Cout), jnp.float32),
            pltpu.SemaphoreType.DMA((nc - 1,)),
            pltpu.SemaphoreType.DMA((1,)),
            pltpu.SemaphoreType.DMA((2,)),
            pltpu.SemaphoreType.DMA((1,)),
            pltpu.SemaphoreType.DMA((2,)),
        ],
        compiler_params=pltpu.CompilerParams(
            vmem_limit_bytes=116 * 1024 * 1024,
            disable_bounds_checks=True,
            disable_semaphore_checks=True,
        ),
    )(x.reshape(2 * T, S, Cin), w.reshape(Cin, Cout), b)
    return out.reshape(B, H, W, Cout)
```

```python
import jax
import jax.numpy as jnp
import jax.experimental.pallas as pl
import jax.experimental.pallas.tpu as pltpu

S = 4096
T = 6
AR, RR = 3, 16
WPAT = (48, 40, 40)
QA = 128
QB = 256
PRE = 3
LROWS = 96
W0 = 21
KB = 3
WSPLIT = 8


@jax.jit
def pallas_standalone__standard_2d_1d_3d_conv__vision_kernel(
    x: jax.Array,
    w: jax.Array,
    b: jax.Array,
):
    B, H, W, Cin = x.shape
    Cout = w.shape[-1]
    assert w.shape[:2] == (1, 1) and Cin == Cout
    M = B * H * W
    P = sum(WPAT)
    assert M % (2 * T * S) == 0 and T % AR == 0 and Cin % WSPLIT == 0
    assert S % QB == 0 and QB % QA == 0 and QB % P == 0 and QA % RR == 0
    assert LROWS % RR == 0 and 0 < LROWS < QA
    nh = M // (2 * T * S)
    nc = nh * S // QA
    ncb = nh * S // QB
    nu = nh * S // P
    cb0 = (nc - 2) * QA // QB
    n_a = cb0 * QB // QA
    n_b = 2 * ncb - cb0
    wend = W0 + KB * n_b
    assert PRE < nc <= n_a + PRE
    assert W0 <= cb0 * QB // P and wend <= 2 * nu
    assert all(W0 + KB * n <= (cb0 + n) * QB // P for n in range(1, n_b + 1))
    wrows = Cin // WSPLIT
    last, tail = S - QA, S - LROWS

    def kernel_function(x_hbm, w_hbm, b_hbm, o_hbm,
                        buf, w_ref, b_ref, bf_ref, rsem, hsem, lsem, wsem, psem):
        def split(c, n):
            h = (c >= n).astype(jnp.int32)
            return h, c - h * n

        def locate(c, size):
            g = jax.lax.div(c, S // size)
            return g, pl.multiple_of((c - g * (S // size)) * size, size)

        def stream0(h, g):
            return (h * nh + g) * T

        def start_round(g, row, sems):
            for s in range(0, T, AR):
                for h in range(2):
                    idx = (pl.ds(stream0(h, g) + s, AR), pl.ds(row, RR), slice(None))
                    pltpu.make_async_copy(
                        x_hbm.at[idx], buf.at[idx], sems[h]).start(priority=h)

        def start_chunk(c):
            g, row = locate(c, QA)
            for t in range(0, QA, RR):
                start_round(g, pl.multiple_of(row + t, RR), (rsem.at[c], hsem.at[g]))

        def start_last_chunk():
            for row in range(last, S, RR):
                k = 0 if row < tail else 2
                start_round(nh - 1, row, (lsem.at[k], lsem.at[k + 1]))

        def wait_reads(h, g, row, nrows, sem):
            v = buf.at[pl.ds(stream0(h, g), T), pl.ds(row, nrows), :]
            pltpu.make_async_copy(v, v, sem).wait()

        def start_write_unit(u):
            h, uu = split(u, nu)
            g, row = locate(uu, P)
            off = 0
            for n in WPAT:
                idx = (pl.ds(stream0(h, g), T),
                       pl.ds(pl.multiple_of(row + off, 8), n), slice(None))
                pltpu.make_async_copy(buf.at[idx], o_hbm.at[idx], wsem.at[0]).start()
                off += n

        def matmul_in_place(h, c, size):
            g, row = locate(c, size)
            idx = (pl.ds(stream0(h, g), T), pl.ds(row, size), slice(None))
            acc = jnp.dot(buf[idx].reshape(T * size, Cin), w_ref[...],
                          preferred_element_type=jnp.float32)
            buf[idx] = (acc + bf_ref[...]).astype(buf.dtype).reshape(T, size, Cout)

        def loop(lo, hi, fn):
            def body(i, c):
                fn(i)
                return c
            jax.lax.fori_loop(lo, hi, body, 0)

        w_copies = [
            pltpu.make_async_copy(w_hbm.at[pl.ds(k * wrows, wrows)],
                                  w_ref.at[pl.ds(k * wrows, wrows)], psem.at[0])
            for k in range(WSPLIT)
        ]
        b_copy = pltpu.make_async_copy(b_hbm, b_ref, psem.at[1])
        for k, cp in enumerate(w_copies):
            cp.start(priority=k % 2)
        b_copy.start()
        loop(0, PRE, start_chunk)
        b_copy.wait()
        bf_ref[...] = b_ref[...].astype(jnp.float32).reshape(1, Cout)
        for cp in w_copies:
            cp.wait()

        def step_a(i):
            @pl.when(i + PRE < nc - 1)
            def _():
                start_chunk(i + PRE)

            @pl.when(i + PRE == nc - 1)
            def _():
                start_last_chunk()

            wait_reads(0, *locate(i, QA), QA, rsem.at[i])
            matmul_in_place(0, i, QA)

        loop(0, n_a, step_a)

        for c in range(n_a, nc - 1):
            wait_reads(0, c * QA // S, c * QA % S, QA, rsem.at[c])
        for g in range(nh):
            wait_reads(1, g, 0, S if g < nh - 1 else last, hsem.at[g])
        for h in range(2):
            wait_reads(h, nh - 1, last, tail - last, lsem.at[h])
        loop(0, W0, start_write_unit)
        for h in range(2):
            wait_reads(h, nh - 1, tail, S - tail, lsem.at[2 + h])

        def step_b(i):
            matmul_in_place(*split(cb0 + i, ncb), QB)
            for t in range(KB):
                start_write_unit(W0 + i * KB + t)

        loop(0, n_b, step_b)
        loop(wend, 2 * nu, start_write_unit)
        pltpu.make_async_copy(buf, o_hbm, wsem.at[0]).wait()

    out = pl.pallas_call(
        kernel_function,
        in_specs=[pl.BlockSpec(memory_space=pl.ANY)] * 3,
        out_specs=pl.BlockSpec(memory_space=pl.ANY),
        out_shape=jax.ShapeDtypeStruct((M // S, S, Cout), x.dtype),
        scratch_shapes=[
            pltpu.VMEM((M // S, S, Cin), x.dtype),
            pltpu.VMEM((Cin, Cout), w.dtype),
            pltpu.VMEM(b.shape, b.dtype),
            pltpu.VMEM((1, Cout), jnp.float32),
            pltpu.SemaphoreType.DMA((nc - 1,)),
            pltpu.SemaphoreType.DMA((nh,)),
            pltpu.SemaphoreType.DMA((4,)),
            pltpu.SemaphoreType.DMA((1,)),
            pltpu.SemaphoreType.DMA((2,)),
        ],
        compiler_params=pltpu.CompilerParams(
            vmem_limit_bytes=116 * 1024 * 1024,
            disable_bounds_checks=True,
            disable_semaphore_checks=True,
        ),
    )(x.reshape(M // S, S, Cin), w.reshape(Cin, Cout), b)
    return out.reshape(B, H, W, Cout)
```

```python
import jax
import jax.numpy as jnp
import jax.experimental.pallas as pl
import jax.experimental.pallas.tpu as pltpu

S = 4096
T = 6
AR, RR = 3, 16
WR = 40
QA = 128
QB = 256
PRE = 3
LROWS = 96
W0 = 64
KB = 11
WSPLIT = 8


@jax.jit
def pallas_standalone__standard_2d_1d_3d_conv__vision_kernel(
    x: jax.Array,
    w: jax.Array,
    b: jax.Array,
):
    B, H, W, Cin = x.shape
    Cout = w.shape[-1]
    assert w.shape[:2] == (1, 1) and Cin == Cout
    M = B * H * W
    assert M % (2 * T * S) == 0 and T % AR == 0 and Cin % WSPLIT == 0
    assert S % QB == 0 and QB % QA == 0 and QA % RR == 0 and WR % 8 == 0
    assert LROWS % RR == 0 and 0 < LROWS < QA
    nh = M // (2 * T * S)
    nc = nh * S // QA
    ncb = nh * S // QB
    nwg = S // WR
    nw = 2 * nh * nwg
    cb0 = (nc - 2) * QA // QB
    n_a = cb0 * QB // QA
    n_b = 2 * ncb - cb0
    wend = W0 + KB * n_b
    assert PRE < nc <= n_a + PRE

    def write_end(k):
        g, kk = divmod(k, nwg)
        return g * S + (S if kk == nwg - 1 else (kk + 1) * WR)

    assert wend <= nw
    assert all(write_end(W0 + KB * n - 1) <= (cb0 + n) * QB for n in range(n_b + 1))
    wrows = Cin // WSPLIT
    last, tail = S - QA, S - LROWS

    def kernel_function(x_hbm, w_hbm, b_hbm, o_hbm,
                        buf, w_ref, b_ref, bf_ref, rsem, hsem, lsem, wsem, psem):
        def split(c, n):
            h = (c >= n).astype(jnp.int32)
            return h, c - h * n

        def locate(c, size):
            g = jax.lax.div(c, S // size)
            return g, pl.multiple_of((c - g * (S // size)) * size, size)

        def stream0(h, g):
            return (h * nh + g) * T

        def start_round(g, row, sems):
            for s in range(0, T, AR):
                for h in range(2):
                    idx = (pl.ds(stream0(h, g) + s, AR), pl.ds(row, RR), slice(None))
                    pltpu.make_async_copy(
                        x_hbm.at[idx], buf.at[idx], sems[h]).start(priority=h)

        def start_chunk(c):
            g, row = locate(c, QA)
            for t in range(0, QA, RR):
                start_round(g, pl.multiple_of(row + t, RR), (rsem.at[c], hsem.at[g]))

        def start_last_chunk():
            for row in range(last, S, RR):
                k = 0 if row < tail else 2
                start_round(nh - 1, row, (lsem.at[k], lsem.at[k + 1]))

        def wait_reads(h, g, row, nrows, sem):
            v = buf.at[pl.ds(stream0(h, g), T), pl.ds(row, nrows), :]
            pltpu.make_async_copy(v, v, sem).wait()

        def start_write(k):
            g = jax.lax.div(k, nwg)
            kk = k - g * nwg

            def start(row, nrows):
                idx = (pl.ds(stream0(0, g), T), pl.ds(row, nrows), slice(None))
                pltpu.make_async_copy(buf.at[idx], o_hbm.at[idx], wsem.at[0]).start()

            @pl.when(kk < nwg - 1)
            def _():
                start(pl.multiple_of(kk * WR, 8), WR)

            @pl.when(kk == nwg - 1)
            def _():
                start((nwg - 1) * WR, S - (nwg - 1) * WR)

        def matmul_in_place(h, c, size):
            g, row = locate(c, size)
            idx = (pl.ds(stream0(h, g), T), pl.ds(row, size), slice(None))
            acc = jnp.dot(buf[idx].reshape(T * size, Cin), w_ref[...],
                          preferred_element_type=jnp.float32)
            buf[idx] = (acc + bf_ref[...]).astype(buf.dtype).reshape(T, size, Cout)

        def loop(lo, hi, fn):
            def body(i, c):
                fn(i)
                return c
            jax.lax.fori_loop(lo, hi, body, 0)

        w_copies = [
            pltpu.make_async_copy(w_hbm.at[pl.ds(k * wrows, wrows)],
                                  w_ref.at[pl.ds(k * wrows, wrows)], psem.at[0])
            for k in range(WSPLIT)
        ]
        b_copy = pltpu.make_async_copy(b_hbm, b_ref, psem.at[1])
        for k, cp in enumerate(w_copies):
            cp.start(priority=k % 2)
        b_copy.start()
        loop(0, PRE, start_chunk)
        b_copy.wait()
        bf_ref[...] = b_ref[...].astype(jnp.float32).reshape(1, Cout)
        for cp in w_copies:
            cp.wait()

        def step_a(i):
            @pl.when(i + PRE < nc - 1)
            def _():
                start_chunk(i + PRE)

            @pl.when(i + PRE == nc - 1)
            def _():
                start_last_chunk()

            wait_reads(0, *locate(i, QA), QA, rsem.at[i])
            matmul_in_place(0, i, QA)

        loop(0, n_a, step_a)

        for c in range(n_a, nc - 1):
            wait_reads(0, c * QA // S, c * QA % S, QA, rsem.at[c])
        for g in range(nh):
            wait_reads(1, g, 0, S if g < nh - 1 else last, hsem.at[g])
        for h in range(2):
            wait_reads(h, nh - 1, last, tail - last, lsem.at[h])
        loop(0, W0, start_write)
        for h in range(2):
            wait_reads(h, nh - 1, tail, S - tail, lsem.at[2 + h])

        def step_b(i):
            matmul_in_place(*split(cb0 + i, ncb), QB)
            for t in range(KB):
                start_write(W0 + i * KB + t)

        loop(0, n_b, step_b)
        loop(wend, nw, start_write)
        pltpu.make_async_copy(buf, o_hbm, wsem.at[0]).wait()

    out = pl.pallas_call(
        kernel_function,
        in_specs=[pl.BlockSpec(memory_space=pl.ANY)] * 3,
        out_specs=pl.BlockSpec(memory_space=pl.ANY),
        out_shape=jax.ShapeDtypeStruct((M // S, S, Cout), x.dtype),
        scratch_shapes=[
            pltpu.VMEM((M // S, S, Cin), x.dtype),
            pltpu.VMEM((Cin, Cout), w.dtype),
            pltpu.VMEM(b.shape, b.dtype),
            pltpu.VMEM((1, Cout), jnp.float32),
            pltpu.SemaphoreType.DMA((nc - 1,)),
            pltpu.SemaphoreType.DMA((nh,)),
            pltpu.SemaphoreType.DMA((4,)),
            pltpu.SemaphoreType.DMA((1,)),
            pltpu.SemaphoreType.DMA((2,)),
        ],
        compiler_params=pltpu.CompilerParams(
            vmem_limit_bytes=116 * 1024 * 1024,
            disable_bounds_checks=True,
            disable_semaphore_checks=True,
        ),
    )(x.reshape(M // S, S, Cin), w.reshape(Cin, Cout), b)
    return out.reshape(B, H, W, Cout)
```

```python
import jax
import jax.numpy as jnp
import jax.experimental.pallas as pl
import jax.experimental.pallas.tpu as pltpu

S = 4096
T = 6
AR, RR = 3, 16
WR = 40
QA = 128
QB = 256
PRE = 3
LAG = 6
LROWS = 96
W0 = 64
KB = 10
WSPLIT = 8


@jax.jit
def pallas_standalone__standard_2d_1d_3d_conv__vision_kernel(
    x: jax.Array,
    w: jax.Array,
    b: jax.Array,
):
    B, H, W, Cin = x.shape
    Cout = w.shape[-1]
    assert w.shape[:2] == (1, 1) and Cin == Cout
    M = B * H * W
    assert M % (2 * T * S) == 0 and T % AR == 0 and Cin % WSPLIT == 0
    assert S % QB == 0 and QB % QA == 0 and QA % RR == 0 and WR % 8 == 0
    assert LROWS % RR == 0 and 0 < LROWS < QA
    nh = M // (2 * T * S)
    nc = nh * S // QA
    ncb = nh * S // QB
    nwg = S // WR
    nw = 2 * nh * nwg
    cb0 = (nc - LAG) * QA // QB
    n_a = cb0 * QB // QA
    n_b = 2 * ncb - cb0
    wend = W0 + KB * n_b
    assert 0 < n_a and n_a + PRE <= nc - 1

    def write_end(k):
        g, kk = divmod(k, nwg)
        return g * S + (S if kk == nwg - 1 else (kk + 1) * WR)

    assert wend <= nw
    assert all(write_end(W0 + KB * n - 1) <= (cb0 + n) * QB for n in range(n_b + 1))
    wrows = Cin // WSPLIT
    last, tail = S - QA, S - LROWS

    def kernel_function(x_hbm, w_hbm, b_hbm, o_hbm,
                        buf, w_ref, b_ref, bf_ref, rsem, hsem, lsem, wsem, psem):
        def split(c, n):
            h = (c >= n).astype(jnp.int32)
            return h, c - h * n

        def locate(c, size):
            g = jax.lax.div(c, S // size)
            return g, pl.multiple_of((c - g * (S // size)) * size, size)

        def stream0(h, g):
            return (h * nh + g) * T

        def start_round(g, row, sems):
            for s in range(0, T, AR):
                for h in range(2):
                    idx = (pl.ds(stream0(h, g) + s, AR), pl.ds(row, RR), slice(None))
                    pltpu.make_async_copy(
                        x_hbm.at[idx], buf.at[idx], sems[h]).start(priority=h)

        def start_chunk(c):
            g, row = locate(c, QA)
            for t in range(0, QA, RR):
                start_round(g, pl.multiple_of(row + t, RR), (rsem.at[c], hsem.at[g]))

        def start_last_chunk():
            for row in range(last, S, RR):
                k = 0 if row < tail else 2
                start_round(nh - 1, row, (lsem.at[k], lsem.at[k + 1]))

        def wait_reads(h, g, row, nrows, sem):
            v = buf.at[pl.ds(stream0(h, g), T), pl.ds(row, nrows), :]
            pltpu.make_async_copy(v, v, sem).wait()

        def start_write(k):
            g = jax.lax.div(k, nwg)
            kk = k - g * nwg

            def start(row, nrows):
                idx = (pl.ds(stream0(0, g), T), pl.ds(row, nrows), slice(None))
                pltpu.make_async_copy(buf.at[idx], o_hbm.at[idx], wsem.at[0]).start()

            @pl.when(kk < nwg - 1)
            def _():
                start(pl.multiple_of(kk * WR, 8), WR)

            @pl.when(kk == nwg - 1)
            def _():
                start((nwg - 1) * WR, S - (nwg - 1) * WR)

        def matmul_in_place(h, c, size):
            g, row = locate(c, size)
            idx = (pl.ds(stream0(h, g), T), pl.ds(row, size), slice(None))
            acc = jnp.dot(buf[idx].reshape(T * size, Cin), w_ref[...],
                          preferred_element_type=jnp.float32)
            buf[idx] = (acc + bf_ref[...]).astype(buf.dtype).reshape(T, size, Cout)

        def loop(lo, hi, fn):
            def body(i, c):
                fn(i)
                return c
            jax.lax.fori_loop(lo, hi, body, 0)

        w_copies = [
            pltpu.make_async_copy(w_hbm.at[pl.ds(k * wrows, wrows)],
                                  w_ref.at[pl.ds(k * wrows, wrows)], psem.at[0])
            for k in range(WSPLIT)
        ]
        b_copy = pltpu.make_async_copy(b_hbm, b_ref, psem.at[1])
        for k, cp in enumerate(w_copies):
            cp.start(priority=k % 2)
        b_copy.start()
        loop(0, PRE, start_chunk)
        b_copy.wait()
        bf_ref[...] = b_ref[...].astype(jnp.float32).reshape(1, Cout)
        for cp in w_copies:
            cp.wait()

        def step_a(i):
            start_chunk(i + PRE)
            wait_reads(0, *locate(i, QA), QA, rsem.at[i])
            matmul_in_place(0, i, QA)

        loop(0, n_a, step_a)
        loop(n_a + PRE, nc - 1, start_chunk)
        start_last_chunk()

        for c in range(n_a, nc - 1):
            wait_reads(0, c * QA // S, c * QA % S, QA, rsem.at[c])
        for g in range(nh):
            wait_reads(1, g, 0, S if g < nh - 1 else last, hsem.at[g])
        for h in range(2):
            wait_reads(h, nh - 1, last, tail - last, lsem.at[h])
        loop(0, W0, start_write)
        for h in range(2):
            wait_reads(h, nh - 1, tail, S - tail, lsem.at[2 + h])

        def step_b(i):
            matmul_in_place(*split(cb0 + i, ncb), QB)
            for t in range(KB):
                start_write(W0 + i * KB + t)

        loop(0, n_b, step_b)
        loop(wend, nw, start_write)
        pltpu.make_async_copy(buf, o_hbm, wsem.at[0]).wait()

    out = pl.pallas_call(
        kernel_function,
        in_specs=[pl.BlockSpec(memory_space=pl.ANY)] * 3,
        out_specs=pl.BlockSpec(memory_space=pl.ANY),
        out_shape=jax.ShapeDtypeStruct((M // S, S, Cout), x.dtype),
        scratch_shapes=[
            pltpu.VMEM((M // S, S, Cin), x.dtype),
            pltpu.VMEM((Cin, Cout), w.dtype),
            pltpu.VMEM(b.shape, b.dtype),
            pltpu.VMEM((1, Cout), jnp.float32),
            pltpu.SemaphoreType.DMA((nc - 1,)),
            pltpu.SemaphoreType.DMA((nh,)),
            pltpu.SemaphoreType.DMA((4,)),
            pltpu.SemaphoreType.DMA((1,)),
            pltpu.SemaphoreType.DMA((2,)),
        ],
        compiler_params=pltpu.CompilerParams(
            vmem_limit_bytes=116 * 1024 * 1024,
            disable_bounds_checks=True,
            disable_semaphore_checks=True,
        ),
    )(x.reshape(M // S, S, Cin), w.reshape(Cin, Cout), b)
    return out.reshape(B, H, W, Cout)
```

```python
import jax
import jax.numpy as jnp
import jax.experimental.pallas as pl
import jax.experimental.pallas.tpu as pltpu

S = 4096
G = 2
NL, LN = 3, 1368
Q = 152
RPAT = (16, 24, 16, 24, 16, 24, 32)
WPAT = (32, 40, 40, 40)
PRE = 2
LAG = 6
LR = 4
W0 = 5
SKIP = 4
WSPLIT = 8


@jax.jit
def pallas_standalone__standard_2d_1d_3d_conv__vision_kernel(
    x: jax.Array,
    w: jax.Array,
    b: jax.Array,
):
    B, H, W, Cin = x.shape
    Cout = w.shape[-1]
    assert w.shape[:2] == (1, 1) and Cin == Cout
    M = B * H * W
    short = NL * LN - S
    assert M % (2 * G * S) == 0 and LN % Q == 0 and Cin % WSPLIT == 0
    assert sum(RPAT) == Q and sum(WPAT) == Q and 0 < LR < len(RPAT)
    assert 0 < short < min(RPAT[-1], WPAT[-1])
    assert all(v % 8 == 0 for v in (S, LN) + RPAT + WPAT)
    nh = M // (2 * G * S)
    cpg = LN // Q
    nc = nh * cpg
    n_a = nc - LAG
    n_b = 2 * nc - n_a
    assert 0 < n_a and n_a + PRE <= nc - 1

    def issued(n):
        return W0 + 2 * n - n // SKIP

    assert all(issued(n) <= n_a + n for n in range(n_b + 1))
    wrows = Cin // WSPLIT
    early = sum(RPAT[:-LR])

    def kernel_function(x_hbm, w_hbm, b_hbm, o_hbm,
                        buf, w_ref, b_ref, bf_ref, rsem, hsem, lsem, wsem, psem):
        def locate(c):
            if isinstance(c, int):
                return divmod(c, cpg)
            g = jax.lax.div(c, cpg)
            return g, c - g * cpg

        def block(g, j, lane, off, n):
            row = j * Q + (lane * LN + off)
            if not isinstance(row, int):
                row = pl.multiple_of(row, 8)
            return (pl.ds(g * G, G), pl.ds(row, n), slice(None))

        def for_pieces(j, pattern, fn):
            off = 0
            for t, n in enumerate(pattern):
                for lane in range(NL):
                    if lane < NL - 1 or t < len(pattern) - 1:
                        fn(t, lane, off, n)
                    elif isinstance(j, int):
                        fn(t, lane, off, n - short if j == cpg - 1 else n)
                    else:
                        pl.when(j < cpg - 1)(lambda: fn(t, lane, off, n))
                        pl.when(j == cpg - 1)(lambda: fn(t, lane, off, n - short))
                off += n

        def start_reads(c, sems=None):
            g, j = locate(c)

            def start(t, lane, off, n):
                sem = sems(t) if sems else (rsem.at[c], hsem.at[g])
                for h in range(2):
                    idx = block(h * nh + g, j, lane, off, n)
                    pltpu.make_async_copy(
                        x_hbm.at[idx], buf.at[idx], sem[h]).start(priority=h)

            for_pieces(j, RPAT, start)

        def wait_block(idx, sem):
            pltpu.make_async_copy(buf.at[idx], buf.at[idx], sem).wait()

        def wait_reads(c):
            g, j = locate(c)
            for_pieces(j, (Q,), lambda t, lane, off, n: wait_block(
                block(g, j, lane, off, n), rsem.at[c]))

        def start_writes(c):
            g, j = locate(c)

            def start(t, lane, off, n):
                idx = block(g, j, lane, off, n)
                pltpu.make_async_copy(buf.at[idx], o_hbm.at[idx], wsem.at[0]).start()

            for_pieces(j, WPAT, start)

        def matmul_in_place(c):
            g, j = locate(c)
            idx = [block(g, j, lane, 0, Q) for lane in range(NL)]
            xv = jnp.concatenate([buf[i].reshape(G * Q, Cin) for i in idx], axis=0)
            acc = jnp.dot(xv, w_ref[...], preferred_element_type=jnp.float32)
            y = (acc + bf_ref[...]).astype(buf.dtype)
            for lane, i in enumerate(idx):
                buf[i] = y[lane * G * Q:(lane + 1) * G * Q].reshape(G, Q, Cout)

        def loop(lo, hi, fn):
            def body(i, c):
                fn(i)
                return c
            jax.lax.fori_loop(lo, hi, body, 0)

        w_copies = [
            pltpu.make_async_copy(w_hbm.at[pl.ds(k * wrows, wrows)],
                                  w_ref.at[pl.ds(k * wrows, wrows)], psem.at[0])
            for k in range(WSPLIT)
        ]
        b_copy = pltpu.make_async_copy(b_hbm, b_ref, psem.at[1])
        for k, cp in enumerate(w_copies):
            cp.start(priority=k % 2)
        b_copy.start()
        loop(0, PRE, start_reads)
        buf[:, pl.ds(S, short), :] = jnp.zeros((M // S, short, Cin), buf.dtype)
        b_copy.wait()
        bf_ref[...] = b_ref[...].astype(jnp.float32).reshape(1, Cout)
        for cp in w_copies:
            cp.wait()

        def step_a(i):
            start_reads(i + PRE)
            wait_reads(i)
            matmul_in_place(i)

        loop(0, n_a, step_a)
        loop(n_a + PRE, nc - 1, start_reads)
        start_reads(nc - 1, lambda t: (lsem.at[0], lsem.at[1])
                    if t < len(RPAT) - LR else (lsem.at[2], lsem.at[3]))

        for c in range(n_a, nc - 1):
            wait_reads(c)
        for g in range(nh - 1):
            wait_block(block(nh + g, 0, 0, 0, S), hsem.at[g])
        for lane in range(NL):
            wait_block(block(2 * nh - 1, 0, lane, 0, LN - Q), hsem.at[nh - 1])
            for h in range(2):
                wait_block(block(h * nh + nh - 1, cpg - 1, lane, 0, early), lsem.at[h])
        loop(0, W0, start_writes)
        for lane in range(NL):
            n = Q - early - (short if lane == NL - 1 else 0)
            for h in range(2):
                wait_block(block(h * nh + nh - 1, cpg - 1, lane, early, n),
                           lsem.at[2 + h])

        def step_b(i, nxt):
            matmul_in_place(n_a + i)
            start_writes(nxt)
            two = jax.lax.rem(i, SKIP) != SKIP - 1
            pl.when(two)(lambda: start_writes(nxt + 1))
            return nxt + 1 + two.astype(jnp.int32)

        jax.lax.fori_loop(0, n_b, step_b, jnp.int32(W0))
        loop(issued(n_b), 2 * nc, start_writes)
        pltpu.make_async_copy(buf.at[:, pl.ds(0, S), :], o_hbm, wsem.at[0]).wait()

    out = pl.pallas_call(
        kernel_function,
        in_specs=[pl.BlockSpec(memory_space=pl.ANY)] * 3,
        out_specs=pl.BlockSpec(memory_space=pl.ANY),
        out_shape=jax.ShapeDtypeStruct((M // S, S, Cout), x.dtype),
        scratch_shapes=[
            pltpu.VMEM((M // S, NL * LN, Cin), x.dtype),
            pltpu.VMEM((Cin, Cout), w.dtype),
            pltpu.VMEM(b.shape, b.dtype),
            pltpu.VMEM((1, Cout), jnp.float32),
            pltpu.SemaphoreType.DMA((nc - 1,)),
            pltpu.SemaphoreType.DMA((nh,)),
            pltpu.SemaphoreType.DMA((4,)),
            pltpu.SemaphoreType.DMA((1,)),
            pltpu.SemaphoreType.DMA((2,)),
        ],
        compiler_params=pltpu.CompilerParams(
            vmem_limit_bytes=116 * 1024 * 1024,
            disable_bounds_checks=True,
            disable_semaphore_checks=True,
        ),
    )(x.reshape(M // S, S, Cin), w.reshape(Cin, Cout), b)
    return out.reshape(B, H, W, Cout)
```

```python
import jax
import jax.numpy as jnp
import jax.experimental.pallas as pl
import jax.experimental.pallas.tpu as pltpu

S = 4096
G = 2
NL, LN = 3, 1368
Q = 152
RPAT = (16, 24, 16, 24, 16, 24, 32)
WPAT = (32, 40, 40, 40)
PRE = 2
LAG = 6
LR = 4
W0 = 5
SKIP = 4
WSPLIT = 8


@jax.jit
def pallas_standalone__standard_2d_1d_3d_conv__vision_kernel(
    x: jax.Array,
    w: jax.Array,
    b: jax.Array,
):
    B, H, W, Cin = x.shape
    Cout = w.shape[-1]
    assert w.shape[:2] == (1, 1) and Cin == Cout
    M = B * H * W
    short = NL * LN - S
    assert M % (2 * G * S) == 0 and LN % Q == 0 and Cin % WSPLIT == 0
    assert sum(RPAT) == Q and sum(WPAT) == Q and 0 < LR < len(RPAT)
    assert 0 < short < min(RPAT[-1], WPAT[-1])
    assert all(v % 8 == 0 for v in (S, LN) + RPAT + WPAT)
    nh = M // (2 * G * S)
    cpg = LN // Q
    nc = nh * cpg
    n_a = nc - LAG
    n_b = 2 * nc - n_a
    assert 0 < n_a and n_a + PRE <= nc - 1

    def issued(n):
        return W0 + 2 * n - n // SKIP

    assert all(issued(n) <= n_a + n for n in range(n_b + 1))
    wrows = Cin // WSPLIT
    early = sum(RPAT[:-LR])

    def kernel_function(x_hbm, w_hbm, b_hbm, o_hbm,
                        buf, w_ref, b_ref, bf_ref, rsem, hsem, lsem, wsem, psem):
        def locate(c):
            if isinstance(c, int):
                return divmod(c, cpg)
            g = jax.lax.div(c, cpg)
            return g, c - g * cpg

        def block(g, j, lane, off, n):
            row = j * Q + (lane * LN + off)
            if not isinstance(row, int):
                row = pl.multiple_of(row, 8)
            return (pl.ds(g * G, G), pl.ds(row, n), slice(None))

        def for_pieces(j, pattern, fn):
            off = 0
            for t, n in enumerate(pattern):
                for lane in range(NL):
                    if lane < NL - 1 or t < len(pattern) - 1:
                        fn(t, lane, off, n)
                    elif isinstance(j, int):
                        fn(t, lane, off, n - short if j == cpg - 1 else n)
                    else:
                        pl.when(j < cpg - 1)(lambda: fn(t, lane, off, n))
                        pl.when(j == cpg - 1)(lambda: fn(t, lane, off, n - short))
                off += n

        def last_sem(late, h, lane):
            return lsem.at[(2 * late + h) * NL + lane]

        def start_reads(c):
            g, j = locate(c)

            def start(t, lane, off, n):
                for h in range(2):
                    if isinstance(c, int):
                        sem = last_sem(int(t >= len(RPAT) - LR), h, lane)
                    else:
                        sem = (rsem.at[c * NL + lane], hsem.at[g * NL + lane])[h]
                    idx = block(h * nh + g, j, lane, off, n)
                    pltpu.make_async_copy(
                        x_hbm.at[idx], buf.at[idx], sem).start(priority=h)

            for_pieces(j, RPAT, start)

        def wait_block(idx, sem):
            pltpu.make_async_copy(buf.at[idx], buf.at[idx], sem).wait()

        def wait_reads(c):
            g, j = locate(c)
            for_pieces(j, (Q,), lambda t, lane, off, n: wait_block(
                block(g, j, lane, off, n), rsem.at[c * NL + lane]))

        def start_writes(c):
            g, j = locate(c)

            def start(t, lane, off, n):
                idx = block(g, j, lane, off, n)
                pltpu.make_async_copy(buf.at[idx], o_hbm.at[idx], wsem.at[0]).start()

            for_pieces(j, WPAT, start)

        def matmul_in_place(c):
            g, j = locate(c)
            idx = [block(g, j, lane, 0, Q) for lane in range(NL)]
            xv = jnp.concatenate([buf[i].reshape(G * Q, Cin) for i in idx], axis=0)
            acc = jnp.dot(xv, w_ref[...], preferred_element_type=jnp.float32)
            y = (acc + bf_ref[...]).astype(buf.dtype)
            for lane, i in enumerate(idx):
                buf[i] = y[lane * G * Q:(lane + 1) * G * Q].reshape(G, Q, Cout)

        def loop(lo, hi, fn):
            def body(i, c):
                fn(i)
                return c
            jax.lax.fori_loop(lo, hi, body, 0)

        w_copies = [
            pltpu.make_async_copy(w_hbm.at[pl.ds(k * wrows, wrows)],
                                  w_ref.at[pl.ds(k * wrows, wrows)], psem.at[0])
            for k in range(WSPLIT)
        ]
        b_copy = pltpu.make_async_copy(b_hbm, b_ref, psem.at[1])
        for k, cp in enumerate(w_copies):
            cp.start(priority=k % 2)
        b_copy.start()
        loop(0, PRE, start_reads)
        buf[:, pl.ds(S, short), :] = jnp.zeros((M // S, short, Cin), buf.dtype)
        b_copy.wait()
        bf_ref[...] = b_ref[...].astype(jnp.float32).reshape(1, Cout)
        for cp in w_copies:
            cp.wait()

        def step_a(i):
            start_reads(i + PRE)
            wait_reads(i)
            matmul_in_place(i)

        loop(0, n_a, step_a)
        loop(n_a + PRE, nc - 1, start_reads)
        start_reads(nc - 1)

        for c in range(n_a, nc - 1):
            wait_reads(c)
        cut = [short if lane == NL - 1 else 0 for lane in range(NL)]
        for g in range(nh):
            for lane in range(NL):
                n = LN - cut[lane] if g < nh - 1 else LN - Q
                wait_block(block(nh + g, 0, lane, 0, n), hsem.at[g * NL + lane])
        for h in range(2):
            for lane in range(NL):
                wait_block(block(h * nh + nh - 1, cpg - 1, lane, 0, early),
                           last_sem(0, h, lane))
        loop(0, W0, start_writes)
        for h in range(2):
            for lane in range(NL):
                wait_block(
                    block(h * nh + nh - 1, cpg - 1, lane, early, Q - early - cut[lane]),
                    last_sem(1, h, lane))

        def step_b(i, nxt):
            matmul_in_place(n_a + i)
            start_writes(nxt)
            two = jax.lax.rem(i, SKIP) != SKIP - 1
            pl.when(two)(lambda: start_writes(nxt + 1))
            return nxt + 1 + two.astype(jnp.int32)

        jax.lax.fori_loop(0, n_b, step_b, jnp.int32(W0))
        loop(issued(n_b), 2 * nc, start_writes)
        pltpu.make_async_copy(buf.at[:, pl.ds(0, S), :], o_hbm, wsem.at[0]).wait()

    out = pl.pallas_call(
        kernel_function,
        in_specs=[pl.BlockSpec(memory_space=pl.ANY)] * 3,
        out_specs=pl.BlockSpec(memory_space=pl.ANY),
        out_shape=jax.ShapeDtypeStruct((M // S, S, Cout), x.dtype),
        scratch_shapes=[
            pltpu.VMEM((M // S, NL * LN, Cin), x.dtype),
            pltpu.VMEM((Cin, Cout), w.dtype),
            pltpu.VMEM(b.shape, b.dtype),
            pltpu.VMEM((1, Cout), jnp.float32),
            pltpu.SemaphoreType.DMA(((nc - 1) * NL,)),
            pltpu.SemaphoreType.DMA((nh * NL,)),
            pltpu.SemaphoreType.DMA((4 * NL,)),
            pltpu.SemaphoreType.DMA((1,)),
            pltpu.SemaphoreType.DMA((2,)),
        ],
        compiler_params=pltpu.CompilerParams(
            vmem_limit_bytes=116 * 1024 * 1024,
            disable_bounds_checks=True,
            disable_semaphore_checks=True,
        ),
    )(x.reshape(M // S, S, Cin), w.reshape(Cin, Cout), b)
    return out.reshape(B, H, W, Cout)
```
